```python
import os as _os
_os.environ.setdefault("JAX_PLATFORMS", "cpu")
import jax
import jax.numpy as jnp

def _softmax(x, axis=-1):
    return jax.nn.softmax(x, axis=axis)
def _gelu(x):
    return jax.nn.gelu(x, approximate=True)
def _silu(x):
    return jax.nn.silu(x)
def _sigmoid(x):
    return jax.nn.sigmoid(x)
def _layernorm(x, axis=-1, eps=1e-5):
    m = jnp.mean(x, axis=axis, keepdims=True)
    v = jnp.var(x, axis=axis, keepdims=True)
    return (x - m) / jnp.sqrt(v + eps)
def _scatter_add(tgt, idx, src, axis=0):
    return tgt.at[idx].add(src)
def _segment_sum(src, seg, n):
    return jax.ops.segment_sum(src, seg, n)
class _Rng:
    def __init__(self, key):
        self._k = key
    def _next(self):
        self._k, sub = jax.random.split(self._k)
        return sub
    def normal(self, shape):
        return jax.random.normal(self._next(), shape, dtype=jnp.bfloat16)
    def randint(self, lo, hi, shape):
        return jax.random.randint(self._next(), shape, lo, hi, dtype=jnp.int32)
    def uniform(self, shape, lo=0.0, hi=1.0):
        return jax.random.uniform(self._next(), shape, jnp.bfloat16, lo, hi)
    def permutation(self, n):
        return jax.random.permutation(self._next(), n)


kernel_name = 'concat_heads__mha_block_cached__mha_block_cached__near_ridge'

def setup_inputs():
    _rng = _Rng(jax.random.key(int.from_bytes(__import__("os").urandom(4), "little")))
    _w = (lambda a: (lambda t: t.astype(jnp.bfloat16) if jnp.issubdtype(t.dtype, jnp.floating) else t)(jnp.asarray(a)))
    def _A_setup():
        B, Sq, D = 32, 32, 640
        H, Sk, Dh = 32, 32, 128
        return {
            "x": _w((lambda *s: _rng.normal(s) * 0.8)(B, Sq, D)),
            "k_cache": _w((lambda *s: _rng.normal(s) * 0.8)(B, H, Sk, Dh)),
            "v_cache": _w((lambda *s: _rng.normal(s) * 0.05)(B, H, Sk, Dh)),
            "wq": _w((lambda *s: _rng.normal(s) * 0.8)(D, H * Dh) * (D ** -0.5)),
            "wo": _w((lambda *s: _rng.normal(s) * 0.05)(H * Dh, D) * ((H * Dh) ** -0.5)),
        }
    _A_in = _A_setup()

    def _B_setup():
        B, Sq, D = 32, 32, 640
        H, Sk, Dh = 32, 32, 128
        return {
            "x": _w((lambda *s: _rng.normal(s) * 0.8)(B, Sq, D)),
            "k_cache": _w((lambda *s: _rng.normal(s) * 0.8)(B, H, Sk, Dh)),
            "v_cache": _w((lambda *s: _rng.normal(s) * 0.05)(B, H, Sk, Dh)),
            "wq": _w((lambda *s: _rng.normal(s) * 0.8)(D, H * Dh) * (D ** -0.5)),
            "wo": _w((lambda *s: _rng.normal(s) * 0.05)(H * Dh, D) * ((H * Dh) ** -0.5)),
        }
    _B_in = _B_setup()

    return {
        "A_x": _A_in["x"],
        "A_k_cache": _A_in["k_cache"],
        "A_v_cache": _A_in["v_cache"],
        "A_wq": _A_in["wq"],
        "A_wo": _A_in["wo"],
        "B_x": _B_in["x"],
        "B_k_cache": _B_in["k_cache"],
        "B_v_cache": _B_in["v_cache"],
        "B_wq": _B_in["wq"],
        "B_wo": _B_in["wo"],
    }

def reference(A_x, A_k_cache, A_v_cache, A_wq, A_wo, B_x, B_k_cache, B_v_cache, B_wq, B_wo):
    def _A_ref(x, k_cache, v_cache, wq, wo):
        B, Sq, D = x.shape
        H, Dh = 32, 128
        q = (lambda x, *d: x.transpose(*d))((x @ wq).reshape(B, Sq, H, Dh), 0, 2, 1, 3)
        scores = jnp.einsum("bhqd,bhkd->bhqk", q, k_cache) * (Dh ** -0.5)
        p = _softmax(scores, axis=-1)
        o = jnp.einsum("bhqk,bhkd->bhqd", p, v_cache)
        return (lambda x, *d: x.transpose(*d))(o, 0, 2, 1, 3).reshape(B, Sq, H * Dh) @ wo

    def _B_ref(x, k_cache, v_cache, wq, wo):
        B, Sq, D = x.shape
        H, Dh = 32, 128
        q = (lambda x, *d: x.transpose(*d))((x @ wq).reshape(B, Sq, H, Dh), 0, 2, 1, 3)
        scores = jnp.einsum("bhqd,bhkd->bhqk", q, k_cache) * (Dh ** -0.5)
        p = _softmax(scores, axis=-1)
        o = jnp.einsum("bhqk,bhkd->bhqd", p, v_cache)
        return (lambda x, *d: x.transpose(*d))(o, 0, 2, 1, 3).reshape(B, Sq, H * Dh) @ wo

    a = _A_ref(A_x, A_k_cache, A_v_cache, A_wq, A_wo)
    b = _B_ref(B_x, B_k_cache, B_v_cache, B_wq, B_wo)
    return jnp.concatenate([a, b], axis=-1)
```

```python
import contextlib
import functools
import jax
import jax.numpy as jnp
import numpy as np
from jax import lax
import jax.experimental.pallas as pl
import jax.experimental.pallas.tpu as pltpu

NT = (((1,), (1,)), ((), ()))
SCALE = (128 ** -0.5) * 1.4426950408889634
f32 = jnp.float32
bf16 = jnp.bfloat16


def attn_group_T(q4, k4, v4, lane_blk):
    st = lax.dot_general(k4, q4, NT, preferred_element_type=f32)
    c = jnp.where(lane_blk == 0, st[0:32], jnp.where(lane_blk == 1, st[32:64],
                  jnp.where(lane_blk == 2, st[64:96], st[96:128])))
    m = jnp.max(c, axis=0, keepdims=True)
    e = jnp.exp2(c - m)
    l = jnp.sum(e, axis=0, keepdims=True)
    r = pl.reciprocal(l, approx=True)
    r = r * (2.0 - l * r)
    p = (e * r).astype(bf16)
    zero = jnp.zeros_like(p)
    pt = jnp.concatenate([jnp.where(lane_blk == j, p, zero) for j in range(4)], axis=0)
    return jnp.dot(pt.T, v4, preferred_element_type=f32)


def make(reps=1, scopes=False, peel_first=True, stage_always=True, HS=8):
    HG = HS // 2
    W = HG * 128
    NSB = 32 // HS
    NS = 2 * NSB
    sc = (lambda n: jax.named_scope(n)) if scopes else (lambda n: contextlib.nullcontext())

    def kernel(ax, ak, av, awq, awo, bx, bk, bv, bwq, bwo, out_hbm,
               xv, kv, vv, wqv, wov, acc, q0, q1, o0, o1, stg, sems, fsem, xsem, osem):
        step = pl.program_id(0)
        hbm = [(ak, av, awq, awo), (bk, bv, bwq, bwo)]
        last = NS * reps - 1

        def cps(br, s, slot):
            k_h, v_h, wq_h, wo_h = hbm[br]
            h0 = s * HS
            c0 = s * (HS * 128)
            if not isinstance(s, int):
                c0 = pl.multiple_of(c0, HS * 128)
            return [
                pltpu.make_async_copy(wq_h.at[:, pl.ds(c0, HS * 128)], wqv.at[slot], sems.at[slot, 0]),
                pltpu.make_async_copy(k_h.at[:, pl.ds(h0, HS)], kv.at[slot], sems.at[slot, 1]),
                pltpu.make_async_copy(v_h.at[:, pl.ds(h0, HS)], vv.at[slot], sems.at[slot, 2]),
                pltpu.make_async_copy(wo_h.at[pl.ds(c0, HS * 128), :], wov.at[slot], sems.at[slot, 3]),
            ]

        def first_cps():
            d = {}
            for i in range(2):
                d['wq', i] = pltpu.make_async_copy(awq.at[:, pl.ds(i * W, W)], wqv.at[0, :, pl.ds(i * W, W)], fsem.at[i, 0])
                d['k', i] = pltpu.make_async_copy(ak.at[:, pl.ds(i * HG, HG)], kv.at[0, :, pl.ds(i * HG, HG)], fsem.at[i, 1])
                d['v', i] = pltpu.make_async_copy(av.at[:, pl.ds(i * HG, HG)], vv.at[0, :, pl.ds(i * HG, HG)], fsem.at[i, 2])
                d['wo', i] = pltpu.make_async_copy(awo.at[pl.ds(i * W, W), :], wov.at[0, pl.ds(i * W, W), :], fsem.at[i, 3])
            return d

        xcp = [pltpu.make_async_copy(ax, xv.at[0], xsem.at[0]), pltpu.make_async_copy(bx, xv.at[1], xsem.at[1])]
        sm = step % NS
        br = sm // NSB
        slot = step % 2

        def start_next():
            nxt = (step + 1) % NS
            nb = nxt // NSB
            ns = nxt % NSB

            @pl.when(jnp.logical_and(step < last, nb == 0))
            def _():
                for c in cps(0, ns, 1 - slot): c.start()

            @pl.when(jnp.logical_and(step < last, nb == 1))
            def _():
                for c in cps(1, ns, 1 - slot): c.start()

        def qproj(i, q_sc, slot, br):
            q = jnp.dot(xv[br], wqv[slot, :, i * W:(i + 1) * W], preferred_element_type=f32)
            q_sc[...] = (q * SCALE).astype(bf16)

        def attn(i, q_sc, o_sc, slot):
            aux = lax.broadcasted_iota(jnp.int32, (32, 128), 1) // 32
            for hh in range(HG):
                for g in range(8):
                    q4 = q_sc[g * 128:(g + 1) * 128, hh * 128:(hh + 1) * 128]
                    k4 = kv[slot, 4 * g:4 * g + 4, i * HG + hh].reshape(128, 128)
                    v4 = vv[slot, 4 * g:4 * g + 4, i * HG + hh].reshape(128, 128)
                    o = attn_group_T(q4, k4, v4, aux)
                    o_sc[g * 128:(g + 1) * 128, hh * 128:(hh + 1) * 128] = o.astype(bf16)

        def oproj(i, o_sc, slot, br, final):
            r = acc[br] + jnp.dot(o_sc[...], wov[slot, i * W:(i + 1) * W, :], preferred_element_type=f32)
            acc[br] = r
            if final and stage_always:
                stg[br] = r.astype(bf16)

        def main_body():
            with sc('m_wait'):
                for c in cps(0, 0, slot): c.wait()
                start_next()

                @pl.when(step == (1 if peel_first else 0))
                def _():
                    xcp[1].start()

                @pl.when(step == NSB)
                def _():
                    xcp[1].wait()
            qproj(0, q0, slot, br)
            qproj(1, q1, slot, br)
            attn(0, q0, o0, slot)
            oproj(0, o0, slot, br, False)
            attn(1, q1, o1, slot)
            oproj(1, o1, slot, br, True)

        def first_body():
            d = first_cps()
            with sc('f_w1'):
                xcp[0].start(); d['wq', 0].start()
                acc[...] = jnp.zeros_like(acc)
                xcp[0].wait(); d['wq', 0].wait()
                d['k', 0].start(); d['v', 0].start(); d['wq', 1].start()
            with sc('f_p1'):
                qproj(0, q0, 0, 0)
            with sc('f_w2'):
                d['k', 0].wait(); d['v', 0].wait(); d['wq', 1].wait()
                d['wo', 0].start(); d['k', 1].start(); d['v', 1].start(); d['wo', 1].start()
            with sc('f_p2'):
                qproj(1, q1, 0, 0)
                attn(0, q0, o0, 0)
            with sc('f_w3'):
                d['wo', 0].wait(); d['k', 1].wait(); d['v', 1].wait(); d['wo', 1].wait()
                for c in cps(0, 1, 1): c.start()
            with sc('f_p3'):
                oproj(0, o0, 0, 0, False)
                attn(1, q1, o1, 0)
                oproj(1, o1, 0, 0, True)

        if peel_first:
            pl.when(step == 0)(first_body)
            pl.when(step > 0)(main_body)
        else:
            @pl.when(step == 0)
            def _():
                xcp[0].start()
                for c in cps(0, 0, 0): c.start()
                acc[...] = jnp.zeros_like(acc)
                xcp[0].wait()
            main_body()

        with sc('s_final'):
            for b in range(2):
                oc = pltpu.make_async_copy(stg.at[b], out_hbm.at[:, pl.ds(b * 640, 640)], osem.at[b])

                @pl.when(step == (NSB - 1 if b == 0 else last))
                def _():
                    if not stage_always:
                        stg[b] = acc[b].astype(bf16)
                    oc.start()

            @pl.when(step == last)
            def _():
                for b in range(2):
                    pltpu.make_async_copy(stg.at[b], out_hbm.at[:, pl.ds(b * 640, 640)], osem.at[b]).wait()

    @jax.jit
    def fn(A_x, A_k_cache, A_v_cache, A_wq, A_wo, B_x, B_k_cache, B_v_cache, B_wq, B_wo):
        B, Sq, D = A_x.shape
        H, Sk, Dh = A_k_cache.shape[1:]
        M = B * Sq
        anyspec = pl.BlockSpec(memory_space=pl.ANY)
        V = pltpu.VMEM
        S = pltpu.SemaphoreType.DMA
        scratch = [V((2, M, D), bf16), V((2, B, HS, Sk, Dh), bf16), V((2, B, HS, Sk, Dh), bf16),
                   V((2, D, HS * 128), bf16), V((2, HS * 128, D), bf16), V((2, M, D), f32)] \
            + [V((M, W), bf16)] * 4 + [V((2, M, D), bf16)] + [S((2, 4)), S((2, 4)), S((2,)), S((2,))]
        out = pl.pallas_call(
            kernel,
            grid=(NS * reps,),
            in_specs=[anyspec] * 10,
            out_specs=anyspec,
            out_shape=jax.ShapeDtypeStruct((M, 2 * D), bf16),
            scratch_shapes=scratch,
            compiler_params=pltpu.CompilerParams(
                dimension_semantics=("arbitrary",), vmem_limit_bytes=100 * 1024 * 1024),
        )(A_x.reshape(M, D), A_k_cache, A_v_cache, A_wq, A_wo,
          B_x.reshape(M, D), B_k_cache, B_v_cache, B_wq, B_wo)
        return out.reshape(B, Sq, 2 * D)
    return fn


_impl = make()


@jax.jit
def pallas_concat_heads__mha_block_cached__mha_block_cached__near_ridge_kernel(
    A_x, A_k_cache, A_v_cache, A_wq, A_wo, B_x, B_k_cache, B_v_cache, B_wq, B_wo):
    return _impl(A_x, A_k_cache, A_v_cache, A_wq, A_wo, B_x, B_k_cache, B_v_cache, B_wq, B_wo)
```

```python
import jax
import jax.numpy as jnp
from jax import lax
import jax.experimental.pallas as pl
import jax.experimental.pallas.tpu as pltpu

f32 = jnp.float32
bf16 = jnp.bfloat16

DH = 128
HG = 4
W = HG * DH
RC = 256
NCH = 4
NITEM = 8
NSTEP = 8
QK_SCALE = (DH ** -0.5) * 1.4426950408889634
_NT = (((1,), (1,)), ((), ()))

MAIN_PROG = ("Q0 H Q1 K0 Q2 V0 K1 Q3 V1 K2 N0 V2 K3 N1 V3 K4 N2 V4 K5 N3 V5 "
             "K6 O0 V6 K7 O1 V7 O2 O3 O4 O5 O6 O7")
LAST_PROG = ("Q0 Q1 K0 Q2 V0 K1 Q3 V1 K2 O0 V2 K3 O1 V3 K4 O2 V4 K5 O3 V5 "
             "K6 K7 V6 V7 O4 O5 O6 O7")
FIRST_PHASES = (
    ("x0 wq0 | x1 | wq1 | k0 | v0 | wq2 | k1 | v1 | wo0 | wo1 zero", "x0 wq0", "P0 P1"),
    ("", "x1 wq1", ""),
    ("next wq3 wq4", "", "P2 P3 Q0 Q1 Q2 Q3"),
    ("", "wq2 k0 v0", "K0 K1 V0 N0 K2 V1 N1 K3 V2 N2 V3 N3"),
    ("", "k1 v1 wo0 wo1", "K4 O0 V4 K5 O1 V5 K6 O2 V6 K7 O3 V7 O4 O5 O6 O7"),
)


def _scores(q4, k4, lane_blk):
    st = lax.dot_general(k4, q4, _NT, preferred_element_type=f32)
    return jnp.where(lane_blk == 0, st[0:32],
                     jnp.where(lane_blk == 1, st[32:64],
                               jnp.where(lane_blk == 2, st[64:96], st[96:128])))


def _softmax_keys(s):
    m = jnp.max(s, axis=0, keepdims=True)
    e = jnp.exp2(s - m)
    l = jnp.sum(e, axis=0, keepdims=True)
    r = pl.reciprocal(l, approx=True)
    r = r * (2.0 - l * r)
    return (e * r).astype(bf16)


def _block_diag(p, keep):
    rep = jnp.concatenate([p] * 4, axis=0).T
    u = pltpu.bitcast(rep, jnp.uint32)
    u = jnp.where(keep, u, jnp.zeros_like(u))
    return pltpu.bitcast(u, bf16)


def _kernel(ax, ak, av, awq, awo, bx, bk, bv, bwq, bwo, out_hbm,
            xv, kv, vv, wqv, wov, acc, qv, ov, stg, ssem, qsem, fsem, xsem, osem):
    step = pl.program_id(0)
    last = NSTEP - 1
    hbm = ((ak, av, awq, awo), (bk, bv, bwq, bwo))
    shr = lax.shift_right_logical
    band = lax.bitwise_and

    def step_copies(br, s, slot):
        k_h, v_h, _, wo_h = hbm[br]
        r0 = s * (2 * W)
        if not isinstance(s, int):
            r0 = pl.multiple_of(r0, 2 * W)
        heads = pl.ds(s * (2 * HG), 2 * HG)
        return (
            pltpu.make_async_copy(k_h.at[:, heads], kv.at[slot], ssem.at[slot, 0]),
            pltpu.make_async_copy(v_h.at[:, heads], vv.at[slot], ssem.at[slot, 1]),
            pltpu.make_async_copy(wo_h.at[pl.ds(r0, 2 * W), :], wov.at[slot], ssem.at[slot, 2]),
        )

    def step_wait(slot):
        for i, buf in enumerate((kv, vv, wov)):
            pltpu.make_async_copy(buf.at[slot], buf.at[slot], ssem.at[slot, i]).wait()

    def wq_copy(br, j):
        c0 = j * W
        if not isinstance(j, int):
            c0 = pl.multiple_of(c0, W)
        return pltpu.make_async_copy(hbm[br][2].at[:, pl.ds(c0, W)], wqv.at[j], qsem.at[j])

    def wq_wait(j):
        pltpu.make_async_copy(wqv.at[j], wqv.at[j], qsem.at[j]).wait()

    xb_copy = pltpu.make_async_copy(bx, xv.at[1], xsem.at[0])

    def out_copy(br, c):
        r = pl.ds(c * RC, RC)
        return pltpu.make_async_copy(stg.at[br, r], out_hbm.at[r, pl.ds(br * 640, 640)],
                                     osem.at[br, c])

    def rows(c):
        return slice(c * RC, (c + 1) * RC)

    def cols(item):
        return slice(item * W, (item + 1) * W)

    def q_proj(br, j, item, c):
        q = jnp.dot(xv[br, rows(c), :], wqv[j], preferred_element_type=f32)
        qv[rows(c), cols(item)] = (q * QK_SCALE).astype(bf16)

    def groups(item, c):
        return [(g, h) for g in range(c * RC // 128, (c + 1) * RC // 128)
                for h in range(item * HG, (item + 1) * HG)]

    def tile(g, h):
        return slice(g * 128, (g + 1) * 128), slice(h * DH, (h + 1) * DH)

    def qk_softmax(slot, item, c):
        lane_blk = lax.broadcasted_iota(jnp.int32, (32, 128), 1) // 32
        return [_softmax_keys(_scores(qv[tile(g, h)],
                                      kv[slot, 4 * g:4 * g + 4, h].reshape(128, DH), lane_blk))
                for g, h in groups(item, c)]

    def pv(slot, item, c, ps):
        keep = (lax.broadcasted_iota(jnp.int32, (64, 128), 0) // 16
                == lax.broadcasted_iota(jnp.int32, (64, 128), 1) // 32)
        for (g, h), p in zip(groups(item, c), ps):
            o = jnp.dot(_block_diag(p, keep), vv[slot, 4 * g:4 * g + 4, h].reshape(128, DH),
                        preferred_element_type=f32)
            ov[tile(g, h)] = o.astype(bf16)

    def out_proj(br, slot, item, c, init, emit, keep_acc):
        r = jnp.dot(ov[rows(c), cols(item)], wov[slot, cols(item), :], preferred_element_type=f32)
        if not init:
            r = r + acc[br, rows(c), :]
        if keep_acc:
            acc[br, rows(c), :] = r
        if emit is not None:
            stg[br, rows(c), :] = r.astype(bf16)
            emit(c)

    def run(prog, br, slot, j1, nbr, jn, hook=None, init=False, emit=None, final=False):
        ps = {}
        for tok in prog.split():
            op = tok[0]
            t = int(tok[1:]) if len(tok) > 1 else None
            if op == "P":
                q_proj(br, j1 - 1, 0, t)
            elif op == "Q":
                q_proj(br, j1, 1, t)
            elif op == "N":
                q_proj(nbr, jn, 0, t)
            elif op == "K":
                ps[t] = qk_softmax(slot, t // NCH, t % NCH)
            elif op == "V":
                pv(slot, t // NCH, t % NCH, ps.pop(t))
            elif op == "O":
                item = t // NCH
                out_proj(br, slot, item, t % NCH, init and item == 0,
                         emit if item == 1 else None, not (final and item == 1))
            else:
                hook()
        assert not ps

    def first_body():
        half_m = xv.shape[1] // 2

        def x_part(i):
            r = pl.ds(i * half_m, half_m)
            return pltpu.make_async_copy(ax.at[r], xv.at[0, r], fsem.at[i])

        def cache_part(src, dst, item, j):
            h = pl.ds(item * HG, HG)
            return pltpu.make_async_copy(src.at[:, h], dst.at[0, :, h], fsem.at[j])

        def wo_part(item, j):
            r = pl.ds(item * W, W)
            return pltpu.make_async_copy(awo.at[r, :], wov.at[0, r, :], fsem.at[j])

        cp = {"x0": x_part(0), "x1": x_part(1),
              "k0": cache_part(ak, kv, 0, 2), "v0": cache_part(av, vv, 0, 3),
              "k1": cache_part(ak, kv, 1, 4), "v1": cache_part(av, vv, 1, 5),
              "wo0": wo_part(0, 6), "wo1": wo_part(1, 7)}
        for j in range(5):
            cp[f"wq{j}"] = wq_copy(0, j)

        def zero_rows(i, carry):
            r0 = pl.multiple_of(i * 64, 64)
            acc[1, pl.ds(r0, 64), :] = jnp.zeros((64, acc.shape[2]), f32)
            return carry

        for starts, waits, prog in FIRST_PHASES:
            for n in starts.split():
                if n == "next":
                    for c in step_copies(0, 1, 1):
                        c.start()
                elif n == "zero":
                    lax.fori_loop(0, acc.shape[1] // 64, zero_rows, 0)
                elif n == "|":
                    pl.delay(1)
                else:
                    cp[n].start()
            for n in waits.split():
                cp[n].wait()
            run(prog, 0, 0, 1, 0, 2, init=True)

    def main_body():
        br = shr(step, 2)
        s = band(step, 3)
        slot = band(step, 1)
        j1 = 2 * s + 1
        jn = band(2 * s + 2, NITEM - 1)
        step_wait(slot)
        wq_wait(j1)
        wq_wait(jn)
        pl.when(step == 3)(xb_copy.wait)

        def prefetch():
            nxt = step + 1
            for b in range(2):
                @pl.when(shr(nxt, 2) == b)
                def _():
                    for c in step_copies(b, band(nxt, 3), 1 - slot):
                        c.start()

                for j in (2 * step + 3, 2 * step + 4):
                    @pl.when(shr(j, 3) == b)
                    def _():
                        wq_copy(b, band(j, NITEM - 1)).start()
            pl.when(step == 1)(xb_copy.start)

        def emit(c):
            pl.when(step == 3)(out_copy(0, c).start)

        run(MAIN_PROG, br, slot, j1, shr(step + 1, 2), jn, hook=prefetch, emit=emit)

    def last_body():
        slot = last % 2
        step_wait(slot)
        wq_wait(NITEM - 1)
        run(LAST_PROG, 1, slot, NITEM - 1, None, None,
            emit=lambda c: out_copy(1, c).start(), final=True)
        for b in range(2):
            for c in range(NCH):
                out_copy(b, c).wait()

    pl.when(step == 0)(first_body)
    pl.when(jnp.logical_and(step > 0, step < last))(main_body)
    pl.when(step == last)(last_body)


@jax.jit
def pallas_concat_heads__mha_block_cached__mha_block_cached__near_ridge_kernel(
    A_x: jax.Array,
    A_k_cache: jax.Array,
    A_v_cache: jax.Array,
    A_wq: jax.Array,
    A_wo: jax.Array,
    B_x: jax.Array,
    B_k_cache: jax.Array,
    B_v_cache: jax.Array,
    B_wq: jax.Array,
    B_wo: jax.Array,
):
    B, Sq, D = A_x.shape
    H, Sk, Dh = A_k_cache.shape[1:]
    assert (B, Sq, D, H, Sk, Dh) == (32, 32, 640, 32, 32, DH)
    M = B * Sq
    vmem = pltpu.VMEM
    dma_sem = pltpu.SemaphoreType.DMA
    scratch = [
        vmem((2, M, D), bf16),
        vmem((2, B, 2 * HG, Sk, Dh), bf16),
        vmem((2, B, 2 * HG, Sk, Dh), bf16),
        vmem((NITEM, D, W), bf16),
        vmem((2, 2 * W, D), bf16),
        vmem((2, M, D), f32),
        vmem((M, 2 * W), bf16),
        vmem((M, 2 * W), bf16),
        vmem((2, M, D), bf16),
        dma_sem((2, 3)), dma_sem((NITEM,)), dma_sem((8,)), dma_sem((1,)), dma_sem((2, NCH)),
    ]
    hbm_spec = pl.BlockSpec(memory_space=pl.ANY)
    out = pl.pallas_call(
        _kernel,
        grid=(NSTEP,),
        in_specs=[hbm_spec] * 10,
        out_specs=hbm_spec,
        out_shape=jax.ShapeDtypeStruct((M, 2 * D), bf16),
        scratch_shapes=scratch,
        compiler_params=pltpu.CompilerParams(
            dimension_semantics=("arbitrary",),
            vmem_limit_bytes=100 * 1024 * 1024,
        ),
    )(A_x.reshape(M, D), A_k_cache, A_v_cache, A_wq, A_wo,
      B_x.reshape(M, D), B_k_cache, B_v_cache, B_wq, B_wo)
    return out.reshape(B, Sq, 2 * D)
```

```python
import jax
import jax.numpy as jnp
from jax import lax
import jax.experimental.pallas as pl
import jax.experimental.pallas.tpu as pltpu

f32 = jnp.float32
bf16 = jnp.bfloat16

DH = 128
HG = 4
W = HG * DH
RC = 256
NCH = 4
NITEM = 8
NSTEP = 8
QK_SCALE = (DH ** -0.5) * 1.4426950408889634
_NT = (((1,), (1,)), ((), ()))

MAIN_PROG = ("Q0 H Q1 K0 Q2 V0 K1 Q3 V1 K2 N0 V2 K3 N1 V3 K4 N2 V4 K5 N3 V5 "
             "K6 O0 V6 K7 O1 V7 O2 O3 O4 O5 O6 O7")
LAST_PROG = ("Q0 Q1 K0 Q2 V0 K1 Q3 V1 K2 O0 V2 K3 O1 V3 K4 O2 V4 K5 O3 V5 "
             "K6 E0 V6 K7 E1 V7 E2 E3 E4 E5")
FIRST_START = "x0 w0 | x1 w1 | x2 w2 | wq1 | k0 | v0 | wq2 | k1 | v1 | wo0 | wo1 zero"
FIRST_PHASES = (
    ("x0 w0", "", "S0"),
    ("x1 w1", "", "S1"),
    ("x2 w2", "", "S2"),
    ("wq1", "next wq3 wq4", "Q0 Q1 Q2"),
    ("wq2 k0 v0", "", "K0 Q3 V0 K1 N0 V1 K2 N1 V2 K3 N2 V3 N3"),
    ("k1 v1 wo0 wo1", "", "K4 O0 V4 K5 O1 V5 K6 O2 V6 K7 O3 V7 O4 O5 O6 O7"),
)
KSPLIT = ((0, 128), (128, 384), (384, 640))
OUT_ROWS = (((0, 256), (256, 512), (512, 768), (768, 1024)),
            ((0, 256), (256, 512), (512, 768), (768, 896), (896, 960), (960, 1024)))


def _scores(q4, k4, lane_blk):
    st = lax.dot_general(k4, q4, _NT, preferred_element_type=f32)
    return jnp.where(lane_blk == 0, st[0:32],
                     jnp.where(lane_blk == 1, st[32:64],
                               jnp.where(lane_blk == 2, st[64:96], st[96:128])))


def _softmax_keys(s):
    m = jnp.max(s, axis=0, keepdims=True)
    e = jnp.exp2(s - m)
    l = jnp.sum(e, axis=0, keepdims=True)
    r = pl.reciprocal(l, approx=True)
    r = r * (2.0 - l * r)
    return (e * r).astype(bf16)


def _block_diag(p, keep):
    rep = jnp.concatenate([p] * 4, axis=0).T
    u = pltpu.bitcast(rep, jnp.uint32)
    u = jnp.where(keep, u, jnp.zeros_like(u))
    return pltpu.bitcast(u, bf16)


def _kernel(ax, ak, av, awq, awo, bx, bk, bv, bwq, bwo, out_hbm,
            xv, kv, vv, wqv, wov, acc, qv, ov, stg, ssem, qsem, fsem, xsem, osem):
    step = pl.program_id(0)
    last = NSTEP - 1
    hbm = ((ak, av, awq, awo), (bk, bv, bwq, bwo))
    shr = lax.shift_right_logical
    band = lax.bitwise_and

    def step_copies(br, s, slot):
        k_h, v_h, _, wo_h = hbm[br]
        r0 = s * (2 * W)
        if not isinstance(s, int):
            r0 = pl.multiple_of(r0, 2 * W)
        heads = pl.ds(s * (2 * HG), 2 * HG)
        return (
            pltpu.make_async_copy(k_h.at[:, heads], kv.at[slot], ssem.at[slot, 0]),
            pltpu.make_async_copy(v_h.at[:, heads], vv.at[slot], ssem.at[slot, 1]),
            pltpu.make_async_copy(wo_h.at[pl.ds(r0, 2 * W), :], wov.at[slot], ssem.at[slot, 2]),
        )

    def step_wait(slot):
        for i, buf in enumerate((kv, vv, wov)):
            pltpu.make_async_copy(buf.at[slot], buf.at[slot], ssem.at[slot, i]).wait()

    def wq_copy(br, j):
        c0 = j * W
        if not isinstance(j, int):
            c0 = pl.multiple_of(c0, W)
        return pltpu.make_async_copy(hbm[br][2].at[:, pl.ds(c0, W)], wqv.at[j], qsem.at[j])

    def wq_wait(j):
        pltpu.make_async_copy(wqv.at[j], wqv.at[j], qsem.at[j]).wait()

    xb_copy = pltpu.make_async_copy(bx, xv.at[1], xsem.at[0])

    def out_copy(br, j):
        r0, r1 = OUT_ROWS[br][j]
        d = stg.shape[2]
        return pltpu.make_async_copy(stg.at[br, pl.ds(r0, r1 - r0)],
                                     out_hbm.at[pl.ds(r0, r1 - r0), pl.ds(br * d, d)],
                                     osem.at[br, j])

    def rows(c):
        return slice(c * RC, (c + 1) * RC)

    def cols(item):
        return slice(item * W, (item + 1) * W)

    def q_proj(br, j, item, c):
        q = jnp.dot(xv[br, rows(c), :], wqv[j], preferred_element_type=f32)
        qv[rows(c), cols(item)] = (q * QK_SCALE).astype(bf16)

    def q_proj_first(i):
        k0, k1 = KSPLIT[i]
        q = jnp.dot(xv[0, :, k0:k1], wqv[0, k0:k1, :], preferred_element_type=f32)
        if i > 0:
            q = q + acc[0, :, 0:W]
        if i < len(KSPLIT) - 1:
            acc[0, :, 0:W] = q
        else:
            qv[:, 0:W] = (q * QK_SCALE).astype(bf16)

    def groups(item, c):
        return [(g, h) for g in range(c * RC // 128, (c + 1) * RC // 128)
                for h in range(item * HG, (item + 1) * HG)]

    def tile(g, h):
        return slice(g * 128, (g + 1) * 128), slice(h * DH, (h + 1) * DH)

    def qk_softmax(slot, item, c):
        lane_blk = lax.broadcasted_iota(jnp.int32, (32, 128), 1) // 32
        return [_softmax_keys(_scores(qv[tile(g, h)],
                                      kv[slot, 4 * g:4 * g + 4, h].reshape(128, DH), lane_blk))
                for g, h in groups(item, c)]

    def pv(slot, item, c, ps):
        keep = (lax.broadcasted_iota(jnp.int32, (64, 128), 0) // 16
                == lax.broadcasted_iota(jnp.int32, (64, 128), 1) // 32)
        for (g, h), p in zip(groups(item, c), ps):
            o = jnp.dot(_block_diag(p, keep), vv[slot, 4 * g:4 * g + 4, h].reshape(128, DH),
                        preferred_element_type=f32)
            ov[tile(g, h)] = o.astype(bf16)

    def out_proj(br, slot, item, rs, init=False, keep_acc=True, stage=False):
        r = jnp.dot(ov[rs, cols(item)], wov[slot, cols(item), :], preferred_element_type=f32)
        if not init:
            r = r + acc[br, rs, :]
        if keep_acc:
            acc[br, rs, :] = r
        if stage:
            stg[br, rs, :] = r.astype(bf16)

    def run(prog, br, slot, j1, nbr, jn, hook=None, init=False, emit=None):
        ps = {}
        for tok in prog.split():
            op = tok[0]
            t = int(tok[1:]) if len(tok) > 1 else None
            if op == "S":
                q_proj_first(t)
            elif op == "Q":
                q_proj(br, j1, 1, t)
            elif op == "N":
                q_proj(nbr, jn, 0, t)
            elif op == "K":
                ps[t] = qk_softmax(slot, t // NCH, t % NCH)
            elif op == "V":
                pv(slot, t // NCH, t % NCH, ps.pop(t))
            elif op == "O":
                item, c = divmod(t, NCH)
                stage = emit is not None and item == 1
                out_proj(br, slot, item, rows(c), init=init and item == 0, stage=stage)
                if stage:
                    emit(c)
            elif op == "E":
                out_proj(1, slot, 1, slice(*OUT_ROWS[1][t]), keep_acc=False, stage=True)
                out_copy(1, t).start()
            else:
                hook()
        assert not ps

    def first_body():
        def cache_part(src, dst, item, j):
            h = pl.ds(item * HG, HG)
            return pltpu.make_async_copy(src.at[:, h], dst.at[0, :, h], fsem.at[j])

        def wo_part(item, j):
            r = pl.ds(item * W, W)
            return pltpu.make_async_copy(awo.at[r, :], wov.at[0, r, :], fsem.at[j])

        cp = {"k0": cache_part(ak, kv, 0, 0), "v0": cache_part(av, vv, 0, 1),
              "k1": cache_part(ak, kv, 1, 2), "v1": cache_part(av, vv, 1, 3),
              "wo0": wo_part(0, 4), "wo1": wo_part(1, 5)}
        for j in range(1, 5):
            cp[f"wq{j}"] = wq_copy(0, j)
        for i, (k0, k1) in enumerate(KSPLIT):
            ks = pl.ds(k0, k1 - k0)
            cp[f"x{i}"] = pltpu.make_async_copy(ax.at[:, ks], xv.at[0, :, ks], xsem.at[1 + i])
            cp[f"w{i}"] = pltpu.make_async_copy(awq.at[ks, pl.ds(0, W)], wqv.at[0, ks, :],
                                                fsem.at[6 + i])

        def zero_rows(i, carry):
            r0 = pl.multiple_of(i * 64, 64)
            acc[1, pl.ds(r0, 64), :] = jnp.zeros((64, acc.shape[2]), f32)
            return carry

        def start(names):
            for n in names.split():
                if n == "next":
                    for c in step_copies(0, 1, 1):
                        c.start()
                elif n == "zero":
                    lax.fori_loop(0, acc.shape[1] // 64, zero_rows, 0)
                elif n == "|":
                    pl.delay(1)
                else:
                    cp[n].start()

        start(FIRST_START)
        for waits, starts, prog in FIRST_PHASES:
            for n in waits.split():
                cp[n].wait()
            start(starts)
            run(prog, 0, 0, 1, 0, 2, init=True)

    def main_body():
        br = shr(step, 2)
        s = band(step, 3)
        slot = band(step, 1)
        j1 = 2 * s + 1
        jn = band(2 * s + 2, NITEM - 1)
        step_wait(slot)
        wq_wait(j1)
        wq_wait(jn)
        pl.when(step == 3)(xb_copy.wait)

        def prefetch():
            nxt = step + 1
            for b in range(2):
                @pl.when(shr(nxt, 2) == b)
                def _():
                    for c in step_copies(b, band(nxt, 3), 1 - slot):
                        c.start()

                for j in (2 * step + 3, 2 * step + 4):
                    @pl.when(shr(j, 3) == b)
                    def _():
                        wq_copy(b, band(j, NITEM - 1)).start()
            pl.when(step == 1)(xb_copy.start)

        def emit(c):
            pl.when(step == 3)(out_copy(0, c).start)

        run(MAIN_PROG, br, slot, j1, shr(step + 1, 2), jn, hook=prefetch, emit=emit)

    def last_body():
        slot = last % 2
        step_wait(slot)
        wq_wait(NITEM - 1)
        run(LAST_PROG, 1, slot, NITEM - 1, None, None)
        for b in range(2):
            for j in range(len(OUT_ROWS[b])):
                out_copy(b, j).wait()

    pl.when(step == 0)(first_body)
    pl.when(jnp.logical_and(step > 0, step < last))(main_body)
    pl.when(step == last)(last_body)


@jax.jit
def pallas_concat_heads__mha_block_cached__mha_block_cached__near_ridge_kernel(
    A_x: jax.Array,
    A_k_cache: jax.Array,
    A_v_cache: jax.Array,
    A_wq: jax.Array,
    A_wo: jax.Array,
    B_x: jax.Array,
    B_k_cache: jax.Array,
    B_v_cache: jax.Array,
    B_wq: jax.Array,
    B_wo: jax.Array,
):
    B, Sq, D = A_x.shape
    H, Sk, Dh = A_k_cache.shape[1:]
    assert (B, Sq, D, H, Sk, Dh) == (32, 32, 640, 32, 32, DH)
    M = B * Sq
    vmem = pltpu.VMEM
    dma_sem = pltpu.SemaphoreType.DMA
    scratch = [
        vmem((2, M, D), bf16),
        vmem((2, B, 2 * HG, Sk, Dh), bf16),
        vmem((2, B, 2 * HG, Sk, Dh), bf16),
        vmem((NITEM, D, W), bf16),
        vmem((2, 2 * W, D), bf16),
        vmem((2, M, D), f32),
        vmem((M, 2 * W), bf16),
        vmem((M, 2 * W), bf16),
        vmem((2, M, D), bf16),
        dma_sem((2, 3)), dma_sem((NITEM,)), dma_sem((9,)), dma_sem((4,)),
        dma_sem((2, len(OUT_ROWS[1]))),
    ]
    hbm_spec = pl.BlockSpec(memory_space=pl.ANY)
    out = pl.pallas_call(
        _kernel,
        grid=(NSTEP,),
        in_specs=[hbm_spec] * 10,
        out_specs=hbm_spec,
        out_shape=jax.ShapeDtypeStruct((M, 2 * D), bf16),
        scratch_shapes=scratch,
        compiler_params=pltpu.CompilerParams(
            dimension_semantics=("arbitrary",),
            vmem_limit_bytes=100 * 1024 * 1024,
        ),
    )(A_x.reshape(M, D), A_k_cache, A_v_cache, A_wq, A_wo,
      B_x.reshape(M, D), B_k_cache, B_v_cache, B_wq, B_wo)
    return out.reshape(B, Sq, 2 * D)
```
